```python
import os as _os
_os.environ.setdefault("JAX_PLATFORMS", "cpu")
import jax
import jax.numpy as jnp

def _softmax(x, axis=-1):
    return jax.nn.softmax(x, axis=axis)
def _gelu(x):
    return jax.nn.gelu(x, approximate=True)
def _silu(x):
    return jax.nn.silu(x)
def _sigmoid(x):
    return jax.nn.sigmoid(x)
def _layernorm(x, axis=-1, eps=1e-5):
    m = jnp.mean(x, axis=axis, keepdims=True)
    v = jnp.var(x, axis=axis, keepdims=True)
    return (x - m) / jnp.sqrt(v + eps)
def _scatter_add(tgt, idx, src, axis=0):
    return tgt.at[idx].add(src)
def _segment_sum(src, seg, n):
    return jax.ops.segment_sum(src, seg, n)
class _Rng:
    def __init__(self, key):
        self._k = key
    def _next(self):
        self._k, sub = jax.random.split(self._k)
        return sub
    def normal(self, shape):
        return jax.random.normal(self._next(), shape, dtype=jnp.bfloat16)
    def randint(self, lo, hi, shape):
        return jax.random.randint(self._next(), shape, lo, hi, dtype=jnp.int32)
    def uniform(self, shape, lo=0.0, hi=1.0):
        return jax.random.uniform(self._next(), shape, jnp.bfloat16, lo, hi)
    def permutation(self, n):
        return jax.random.permutation(self._next(), n)


kernel_name = 'gated_mix__mha_block__mixer_s_mlp__prompt'

def setup_inputs():
    _rng = _Rng(jax.random.key(int.from_bytes(__import__("os").urandom(4), "little")))
    _w = (lambda a: (lambda t: t.astype(jnp.bfloat16) if jnp.issubdtype(t.dtype, jnp.floating) else t)(jnp.asarray(a)))
    def _A_setup():
        B, S, D, H = 1, 2048, 512, 32
        return {
            "x": _w((lambda *s: _rng.normal(s) * 0.05)(B, S, D)),
            "wqkv": _w((lambda *s: _rng.normal(s) * 0.8)(D, 3 * D)),
            "wo": _w((lambda *s: _rng.normal(s) * 0.05)(D, D)),
        }
    _A_in = _A_setup()

    def _B_setup():
        B, S, D, F = 1, 2048, 512, 1792
        return {
            "x":  _w((lambda *s: _rng.normal(s) * 0.05)(B, S, D)),
            "w1": _w((lambda *s: _rng.normal(s) * 0.2)(D, D) * (D ** -0.5)),
            "w2": _w((lambda *s: _rng.normal(s) * 0.2)(D, D) * (D ** -0.5)),
            "w3": _w((lambda *s: _rng.normal(s) * 0.2)(D, F) * (D ** -0.5)),
            "w4": _w((lambda *s: _rng.normal(s) * 0.2)(F, D) * (F ** -0.5)),
        }
    _B_in = _B_setup()

    return {
        "A_x": _A_in["x"],
        "A_wqkv": _A_in["wqkv"],
        "A_wo": _A_in["wo"],
        "B_x": _B_in["x"],
        "B_w1": _B_in["w1"],
        "B_w2": _B_in["w2"],
        "B_w3": _B_in["w3"],
        "B_w4": _B_in["w4"],
        "gate_w": _w((lambda *s: _rng.normal(s) * 0.05)(512) * 16.0),
    }

def reference(A_x, A_wqkv, A_wo, B_x, B_w1, B_w2, B_w3, B_w4, gate_w):
    def _A_ref(x, wqkv, wo):
        B, S, D = x.shape
        H = 32
        Dh = D // H
        qkv = (lambda x, *d: x.transpose(*d))((x @ wqkv).reshape(B, S, 3, H, Dh), 2, 0, 3, 1, 4)
        q, k, v = qkv[0], qkv[1], qkv[2]
        scores = jnp.einsum("bhqd,bhkd->bhqk", q, k) * (Dh ** -0.5)
        p = _softmax(scores, axis=-1)
        o = jnp.einsum("bhqk,bhkd->bhqd", p, v)
        return (lambda x, *d: x.transpose(*d))(o, 0, 2, 1, 3).reshape(B, S, D) @ wo

    def _B_ref(x, w1, w2, w3, w4):
        B, S, D = x.shape
        h = _gelu(_layernorm(x, axis=-1) @ w1)
        c = D // 4
        g0 = jnp.pad(h[:, :, 0*c:1*c], ((0, 0), (1, 0), (0, 0)))[:, :S, :]
        g1 = jnp.pad(h[:, :, 1*c:2*c], ((0, 0), (0, 1), (0, 0)))[:, 1:, :]
        g2 = jnp.pad(h[:, :, 2*c:3*c], ((0, 0), (2, 0), (0, 0)))[:, :S, :]
        g3 = jnp.pad(h[:, :, 3*c:   ], ((0, 0), (0, 2), (0, 0)))[:, 2:, :]
        hs = jnp.concatenate([g0, g1, g2, g3], axis=-1) @ w2
        x1 = x + hs
        h2 = _gelu(_layernorm(x1, axis=-1) @ w3) @ w4
        return x1 + h2

    x = A_x
    g = _sigmoid((x * gate_w).sum(-1, keepdims=True))
    a = _A_ref(x, A_wqkv, A_wo)
    b = _B_ref(x, B_w1, B_w2, B_w3, B_w4)
    return g * a + (1 - g) * b
```

```python
import math

import jax
import jax.numpy as jnp
import jax.experimental.pallas as pl
import jax.experimental.pallas.tpu as pltpu

S, D, H, DH, F = 2048, 512, 32, 16, 1792
RB = 512
NB = S // RB
KC = 128
NC = S // KC
UNR = 4
SKEW = 2
FC = 256
PAD = 8
SAFE_SCORE = 40.0
SAFE_V = 2.0 ** 40
QSCALE = (DH ** -0.5) * math.log2(math.e)

f32, bf16, u32 = jnp.float32, jnp.bfloat16, jnp.uint32
NT = (((1,), (1,)), ((), ()))
TN = (((0,), (0,)), ((), ()))


def _dot(a, b):
    return jnp.dot(a, b, preferred_element_type=f32)


def _gelu(x):
    c = math.sqrt(2.0 / math.pi)
    return (0.5 * x) * (1.0 + jnp.tanh(x * (c + (c * 0.044715) * (x * x))))


def _layernorm(x):
    d = x - jnp.mean(x, axis=-1, keepdims=True)
    v = jnp.mean(d * d, axis=-1, keepdims=True)
    return d * jax.lax.rsqrt(v + 1e-5)


def _kernel(x_hbm, wqkv_hbm, wo_hbm, w1_hbm, w2_hbm, w3_hbm, w4_hbm, gw_hbm, out_hbm,
            x_s, wqkv_s, wo_s, w1_s, w2_s, w3_s, w4_s, gw_s, wqt_s, wvt_s,
            kr_s, qt_s, vt_s, h_s, b_s, g_s, st_s, ss_s, s_s, ot_s, o_s,
            in_sem, out_sem):
    def rows(i, n=RB):
        return pl.ds(pl.multiple_of(i * n, n), n)

    x_cp = [pltpu.make_async_copy(x_hbm.at[pl.ds(i * RB, RB)], x_s.at[pl.ds(i * RB, RB)],
                                  in_sem.at[i]) for i in range(NB)]
    wqkv_cp, w1_cp, gw_cp, w2_cp, w3_cp, w4_cp, wo_cp = [
        pltpu.make_async_copy(a, b, in_sem.at[NB + i]) for i, (a, b) in enumerate(
            [(wqkv_hbm, wqkv_s), (w1_hbm, w1_s), (gw_hbm, gw_s), (w2_hbm, w2_s),
             (w3_hbm, w3_s), (w4_hbm, w4_s), (wo_hbm, wo_s)])]
    for cp in [x_cp[0], wqkv_cp, w1_cp] + x_cp[1:] + [gw_cp, w2_cp, w3_cp, w4_cp, wo_cp]:
        cp.start()

    h_s[:PAD] = jnp.zeros((PAD, D), f32)
    h_s[PAD + S:] = jnp.zeros((PAD, D), f32)
    wqkv_cp.wait()
    wqt_s[...] = wqkv_s[:, :D].astype(f32).T.astype(bf16)
    wvt_s[...] = wqkv_s[:, 2 * D:].astype(f32).T.astype(bf16)
    w1_cp.wait()

    def phase1(i, carry):
        qn, km, vm = carry
        for j in range(NB):
            @pl.when(i == j)
            def _():
                x_cp[j].wait()
        x = x_s[rows(i), :]
        k = _dot(x, wqkv_s[:, D:2 * D])
        km = jnp.maximum(km, jnp.max(jnp.abs(k).reshape(RB // 8, 8, D), axis=0))
        kp = pltpu.bitcast(k.astype(bf16), u32)
        for h in range(H):
            kg = kp[:, (h // 8) * 128:(h // 8 + 1) * 128]
            if h % 8:
                kg = pltpu.roll(kg, 128 - (h % 8) * DH, 1)
            kr_s[h, rows(i, RB // 2), :] = kg
        qt = lax_dg(wqt_s[...], x, NT) * QSCALE
        qt_s[i] = qt.astype(bf16)
        q2 = jnp.sum((qt * qt).reshape(H, DH, RB), axis=1)
        for j in range(RB // 128):
            qn = jnp.maximum(qn, q2[:, j * 128:(j + 1) * 128])
        vt = lax_dg(wvt_s[...], x, NT)
        vt_s[i] = vt.astype(bf16)
        va = jnp.max(jnp.abs(vt).reshape(H, DH, RB), axis=1)
        for j in range(RB // 128):
            vm = jnp.maximum(vm, va[:, j * 128:(j + 1) * 128])
        xn = _layernorm(x.astype(f32)).astype(bf16)
        h_s[pl.ds(pl.multiple_of(PAD + i * RB, 8), RB), :] = _gelu(_dot(xn, w1_s[...]))
        return qn, km, vm

    qn, km, vm = jax.lax.fori_loop(
        0, NB, phase1, (jnp.zeros((H, 128), f32), jnp.zeros((8, D), f32), jnp.zeros((H, 128), f32)))

    km = jnp.max(km, axis=0, keepdims=True)
    seg = (jax.lax.broadcasted_iota(jnp.int32, (H, D), 1) // DH
           == jax.lax.broadcasted_iota(jnp.int32, (H, D), 0))
    kn = jnp.sum(jnp.where(seg, km * km, 0.0), axis=1, keepdims=True)
    vm = jnp.max(vm, axis=1, keepdims=True)
    ok = ((jnp.max(qn, axis=1, keepdims=True) * kn <= SAFE_SCORE ** 2)
          & (vm <= SAFE_V) & (vm >= 1.0 / SAFE_V))
    safe = jnp.min(jnp.where(ok, 1.0, 0.0)) > 0.5

    gw_cp.wait()
    w2_cp.wait()
    w3_cp.wait()
    w4_cp.wait()

    def phase2(i, carry):
        c = D // 4
        base = pl.multiple_of(i * RB, RB)
        parts = []
        for j, sh in enumerate((-1, 1, -2, 2)):
            w = h_s[pl.ds(base, RB + 2 * PAD), j * c:(j + 1) * c]
            parts.append(w[PAD + sh:PAD + sh + RB].astype(bf16))
        x = x_s[rows(i), :].astype(f32)
        x1 = x + _dot(jnp.concatenate(parts, axis=1), w2_s[...])
        g = jax.nn.sigmoid(jnp.sum(x * gw_s[...].astype(f32), axis=-1, keepdims=True))
        g_s[rows(i), :] = jnp.broadcast_to(g, (RB, 128))
        xn = _layernorm(x1).astype(bf16)
        acc = x1
        for j in range(F // FC):
            t = _gelu(_dot(xn, w3_s[:, j * FC:(j + 1) * FC])).astype(bf16)
            acc = acc + _dot(t, w4_s[j * FC:(j + 1) * FC, :])
        b_s[rows(i), :] = (1.0 - g) * acc
        return carry

    jax.lax.fori_loop(0, NB, phase2, 0)
    wo_cp.wait()

    def head_rows(h):
        return pl.ds(pl.multiple_of(h * DH, DH), DH)

    def scores(qb, h, c):
        k = pltpu.bitcast(kr_s[h, pl.ds(c * KC // 2, KC // 2), :], bf16)[:, :DH]
        return _dot(k, qt_s[qb, head_rows(h), :])

    def v_chunk(h, c):
        return vt_s[c * KC // RB, head_rows(h), pl.ds(c * KC % RB, KC)]

    for c in range(SKEW):
        ss_s[c] = scores(0, 0, c)

    def fast_heads(qb, it):
        n = UNR * NC
        ss = {}
        for i in range(n):
            dh, cn = divmod(i + SKEW, NC)
            hn, qn_ = it * UNR + dh, qb
            if dh == UNR:
                qn_ = jnp.minimum(qb + hn // H, NB - 1)
                hn = hn % H
            ss[i + SKEW] = scores(qn_, hn, cn)
            dh, c = divmod(i, NC)
            h = it * UNR + dh
            p = jnp.exp2(ss[i] if i >= SKEW else ss_s[i])
            if i + SKEW >= n:
                ss_s[i + SKEW - n] = ss[i + SKEW]
            ls = jnp.sum(p.reshape(KC // 8, 8, RB), axis=0)
            ov = _dot(v_chunk(h, c), p.astype(bf16))
            l, o = (ls, ov) if c == 0 else (l + ls, o + ov)
            if c == NC - 1:
                ot_s[head_rows(h), :] = (o / jnp.sum(l, axis=0, keepdims=True)).astype(bf16)

    def safe_head(qb, h):
        m = None
        for c in range(NC):
            s = scores(qb, h, c)
            s_s[c] = s
            mc = jnp.max(s.reshape(KC // 8, 8, RB), axis=0)
            m = mc if c == 0 else jnp.maximum(m, mc)
        m = jnp.max(m, axis=0, keepdims=True)
        for c in range(NC):
            p = jnp.exp2(s_s[c] - m)
            ls = jnp.sum(p.reshape(KC // 8, 8, RB), axis=0)
            ov = _dot(v_chunk(h, c), p.astype(bf16))
            l, o = (ls, ov) if c == 0 else (l + ls, o + ov)
        ot_s[head_rows(h), :] = (o / jnp.sum(l, axis=0, keepdims=True)).astype(bf16)

    def out_cp(qb):
        return pltpu.make_async_copy(o_s.at[rows(qb)], out_hbm.at[rows(qb)], out_sem.at[qb])

    def phase3(qb, carry):
        @pl.when(safe)
        def _():
            jax.lax.fori_loop(0, H // UNR, lambda it, c: (fast_heads(qb, it), c)[1], 0)

        @pl.when(jnp.logical_not(safe))
        def _():
            jax.lax.fori_loop(0, H, lambda h, c: (safe_head(qb, h), c)[1], 0)

        a = lax_dg(ot_s[...], wo_s[...], TN)
        o_s[rows(qb), :] = (g_s[rows(qb), :][:, :1] * a + b_s[rows(qb), :]).astype(bf16)
        out_cp(qb).start()
        return carry

    jax.lax.fori_loop(0, NB, phase3, 0)
    for qb in range(NB):
        out_cp(qb).wait()


def lax_dg(a, b, dims):
    return jax.lax.dot_general(a, b, dims, preferred_element_type=f32)


@jax.jit
def pallas_gated_mix__mha_block__mixer_s_mlp__prompt_kernel(
    A_x: jax.Array,
    A_wqkv: jax.Array,
    A_wo: jax.Array,
    B_x: jax.Array,
    B_w1: jax.Array,
    B_w2: jax.Array,
    B_w3: jax.Array,
    B_w4: jax.Array,
    gate_w: jax.Array,
):
    del B_x
    vm = pltpu.VMEM
    out = pl.pallas_call(
        _kernel,
        out_shape=jax.ShapeDtypeStruct((S, D), bf16),
        in_specs=[pl.BlockSpec(memory_space=pl.ANY)] * 8,
        out_specs=pl.BlockSpec(memory_space=pl.ANY),
        scratch_shapes=[
            vm((S, D), bf16), vm((D, 3 * D), bf16), vm((D, D), bf16), vm((D, D), bf16),
            vm((D, D), bf16), vm((D, F), bf16), vm((F, D), bf16), vm((1, D), bf16),
            vm((D, D), bf16), vm((D, D), bf16),
            vm((H, S // 2, 128), u32), vm((NB, D, RB), bf16), vm((NB, D, RB), bf16),
            vm((S + 2 * PAD, D), f32), vm((S, D), f32), vm((S, 128), f32),
            vm((2, 8, 128), f32), vm((SKEW, KC, RB), f32), vm((NC, KC, RB), f32),
            vm((D, RB), bf16), vm((S, D), bf16),
            pltpu.SemaphoreType.DMA((NB + 7,)), pltpu.SemaphoreType.DMA((NB,)),
        ],
        compiler_params=pltpu.CompilerParams(vmem_limit_bytes=100 * 2**20),
    )(A_x.reshape(S, D), A_wqkv, A_wo, B_w1, B_w2, B_w3, B_w4, gate_w.reshape(1, D))
    return out.reshape(1, S, D)
```

```python
import math

import jax
import jax.numpy as jnp
import jax.experimental.pallas as pl
import jax.experimental.pallas.tpu as pltpu

S, D, H, DH, F = 2048, 512, 32, 16, 1792
RB = 512
NB = S // RB
KC = 128
NC = S // KC
UNR = 8
NG = H // UNR
SKEW = 2
VK = (0,) + (16,) * 15
VKM = max(VK)
VSKEW = 2
ND = 8
FC = 256
PAD = 8
XP = ((0, 512), (512, 512), (1024, 1024))
SAFE_SCORE = 60.0
SAFE_V = 2.0 ** 30
QSCALE = (DH ** -0.5) * math.log2(math.e)

f32, bf16, u32 = jnp.float32, jnp.bfloat16, jnp.uint32
NT = (((1,), (1,)), ((), ()))
TN = (((0,), (0,)), ((), ()))


def _dot(a, b):
    return jnp.dot(a, b, preferred_element_type=f32)


def _dg(a, b, dims):
    return jax.lax.dot_general(a, b, dims, preferred_element_type=f32)


def _gelu(x):
    c = math.sqrt(2.0 / math.pi)
    return (0.5 * x) * (1.0 + jnp.tanh(x * (c + (c * 0.044715) * (x * x))))


def _layernorm(x):
    d = x - jnp.mean(x, axis=-1, keepdims=True)
    v = jnp.mean(d * d, axis=-1, keepdims=True)
    return d * jax.lax.rsqrt(v + 1e-5)


def _kernel(x_hbm, wqkv_hbm, wo_hbm, w1_hbm, w2_hbm, w3_hbm, w4_hbm, gw_hbm, out_hbm,
            x_s, wqkv_s, wo_s, w1_s, w2_s, w3_s, w4_s, gw_s, wqt_s, wvt_s,
            kr_s, kf_s, qt_s, qf_s, vt_s, h_s, b_s, g_s, st_s, ss_s, s_s, ot_s, o_s,
            x_sem, in_sem, out_sem):
    def rows(i, n=RB):
        return pl.ds(pl.multiple_of(i * n, n), n)

    def cols(j):
        return pltpu.make_async_copy(wqkv_hbm.at[:, pl.ds(j * D, D)], wqkv_s.at[j], in_sem.at[j])

    x_cp = [pltpu.make_async_copy(x_hbm.at[pl.ds(r, n)], x_s.at[pl.ds(r, n)], x_sem.at[i])
            for i, (r, n) in enumerate(XP)]
    wq_cp, wk_cp, wv_cp = cols(0), cols(1), cols(2)
    w1_cp, gw_cp, w2_cp, w3_cp, w4_cp, wo_cp = [
        pltpu.make_async_copy(a, b, in_sem.at[3 + i]) for i, (a, b) in enumerate(
            [(w1_hbm, w1_s), (gw_hbm, gw_s), (w2_hbm, w2_s),
             (w3_hbm, w3_s), (w4_hbm, w4_s), (wo_hbm, wo_s)])]

    def start(*cps):
        for cp in cps:
            cp.start()

    start(x_cp[0], wk_cp)
    h_s[:PAD] = jnp.zeros((PAD, D), f32)
    h_s[PAD + S:] = jnp.zeros((PAD, D), f32)
    ot_s[...] = jnp.zeros(ot_s.shape, bf16)
    x_cp[0].wait()
    wk_cp.wait()
    start(w1_cp, x_cp[1], x_cp[2], wq_cp, wv_cp, gw_cp, w2_cp, w3_cp, w4_cp, wo_cp)

    def proj_k(i, km):
        k = _dot(x_s[i * RB:(i + 1) * RB, :], wqkv_s[1])
        kp = pltpu.bitcast(k.astype(bf16), u32)
        for j in range(H // 8):
            kr_s[8 * j, i * RB // 2:(i + 1) * RB // 2, :] = kp[:, j * 128:(j + 1) * 128]
        return jnp.maximum(km, jnp.max(jnp.abs(k).reshape(RB // 8, 8, D), axis=0))

    def proj_q(i, qn):
        qt = _dg(wqt_s[...], x_s[i * RB:(i + 1) * RB, :], NT) * QSCALE
        qt = qt.astype(bf16)
        qt_s[i] = qt
        qt = qt.astype(f32)
        for j in range(RB // 128):
            qf_s[i, j] = qt[:, j * 128:(j + 1) * 128]
        q2 = jnp.sum((qt * qt).reshape(H, DH, RB), axis=1)
        for j in range(RB // 128):
            qn = jnp.maximum(qn, q2[:, j * 128:(j + 1) * 128])
        return qn

    def proj_h(r, n):
        xn = _layernorm(x_s[r:r + n, :].astype(f32)).astype(bf16)
        h_s[PAD + r:PAD + r + n, :] = _gelu(_dot(xn, w1_s[...]))

    km = proj_k(0, jnp.zeros((8, D), f32))
    w1_cp.wait()
    x_cp[1].wait()
    km = proj_k(1, km)
    for r in range(0, RB, RB // 2):
        proj_h(r, RB // 2)
    for cp in (x_cp[2], wq_cp, wv_cp):
        cp.wait()
    km = proj_k(2, km)
    wqt_s[...] = wqkv_s[0].astype(f32).T.astype(bf16)
    km = proj_k(3, km)
    wvt_s[...] = wqkv_s[2].astype(f32).T.astype(bf16)
    qn = jnp.zeros((H, 128), f32)
    for i in range(NB):
        if i > 0:
            proj_h(i * RB, RB)
        qn = proj_q(i, qn)
    km = jnp.max(km, axis=0, keepdims=True)

    gw_cp.wait()
    w2_cp.wait()
    w3_cp.wait()
    w4_cp.wait()

    def phase2(i, vm):
        vt = _dg(wvt_s[...], x_s[rows(i), :], NT)
        vt_s[i] = vt.astype(bf16)
        va = jnp.max(jnp.abs(vt).reshape(H, DH, RB), axis=1)
        for j in range(RB // 128):
            vm = jnp.maximum(vm, va[:, j * 128:(j + 1) * 128])
        c = D // 4
        hb = RB // 4
        x1s, t0 = [], []
        for r in range(4):
            base = pl.multiple_of(i * RB + r * hb, hb)
            parts = []
            for j, sh in enumerate((-1, 1, -2, 2)):
                w = h_s[pl.ds(base, hb + 2 * PAD), j * c:(j + 1) * c]
                parts.append(w[PAD + sh:PAD + sh + hb].astype(bf16))
            x1s.append(x_s[pl.ds(base, hb), :].astype(f32)
                       + _dot(jnp.concatenate(parts, axis=1), w2_s[...]))
        xns = [_layernorm(x1).astype(bf16) for x1 in x1s]
        t0 = [_dot(xn, w3_s[:, :FC]) for xn in xns]
        x = x_s[rows(i), :].astype(f32)
        g = jax.nn.sigmoid(jnp.sum(x * gw_s[...].astype(f32), axis=-1, keepdims=True))
        g_s[i] = jnp.broadcast_to(g, (RB, 128)).T[:8]
        xn = jnp.concatenate(xns, axis=0)
        acc = jnp.concatenate(x1s, axis=0)
        t = jnp.concatenate(t0, axis=0)
        for j in range(F // FC):
            tn = _dot(xn, w3_s[:, (j + 1) * FC:(j + 2) * FC]) if j + 1 < F // FC else None
            acc = acc + _dot(_gelu(t).astype(bf16), w4_s[j * FC:(j + 1) * FC, :])
            t = tn
            for h in range(j * 5, min(j * 5 + 5, H)):
                kh = kr_s[h // 8 * 8, rows(i, RB // 2), :]
                if h % 8:
                    kh = pltpu.roll(kh, 128 - (h % 8) * DH, 1)
                    kr_s[h, rows(i, RB // 2), :] = kh
                for c in range(RB // KC):
                    kf_s[h, rows(i * (RB // KC) + c, VKM), :] = pltpu.bitcast(
                        kh[((c + 1) * KC - VKM) // 2:(c + 1) * KC // 2], bf16).astype(f32)
        b_s[rows(i), :] = (1.0 - g) * acc
        return vm

    vm = jax.lax.fori_loop(0, NB, phase2, jnp.zeros((H, 128), f32))
    wo_cp.wait()

    seg = (jax.lax.broadcasted_iota(jnp.int32, (H, D), 1) // DH
           == jax.lax.broadcasted_iota(jnp.int32, (H, D), 0))
    kn = jnp.sum(jnp.where(seg, km * km, 0.0), axis=1, keepdims=True)
    vm = jnp.max(vm, axis=1, keepdims=True)
    ok = ((jnp.max(qn, axis=1, keepdims=True) * kn <= SAFE_SCORE ** 2)
          & (vm <= SAFE_V) & (vm >= 1.0 / SAFE_V))
    safe = jnp.min(jnp.where(ok, 1.0, 0.0)) > 0.5

    def head_rows(h):
        return pl.ds(pl.multiple_of(h * DH, DH), DH)

    def scores(qb, h, c, nv=0):
        k = pltpu.bitcast(kr_s[h, pl.ds(c * KC // 2, (KC - nv) // 2), :], bf16)[:, :DH]
        return _dot(k, qt_s[qb, head_rows(h), :])

    def vpu_scores(qb, h, c, deps=None):
        nv = VK[c % len(VK)]
        kf = kf_s[h, (c + 1) * VKM - nv:(c + 1) * VKM, :]
        accs = []
        for d in range(DH):
            if deps is not None and d % (DH // len(deps)) == 0:
                kd = pltpu.bitcast(pltpu.bitcast(kf, u32) | deps[d // (DH // len(deps))], f32)
            elif deps is None:
                kd = kf
            kb = jnp.broadcast_to(kd[:, d:d + 1], (nv, 128))
            for j in range(RB // 128):
                t = kb * jnp.broadcast_to(qf_s[qb, j, pl.ds(h * DH + d, 1), :], (nv, 128))
                accs.append(t if d == 0 else accs[-(RB // 128)] + t)
        return jnp.concatenate(accs[-(RB // 128):], axis=1)

    def finish(qb, h, o, l):
        w = g_s[qb, :1, :] / jnp.sum(l, axis=0, keepdims=True)
        ot_s[head_rows(h), :] = (o * w).astype(bf16)

    def v_chunk(h, c):
        return vt_s[c * KC // RB, head_rows(h), pl.ds(c * KC % RB, KC)]

    for c in range(max(SKEW, VSKEW)):
        nv = VK[c % len(VK)]
        if c < SKEW:
            ss_s[c, :KC - nv] = scores(0, 0, c, nv)
        if nv and c < VSKEW:
            ss_s[c, KC - nv:] = vpu_scores(0, 0, c)

    def project(step, parts=1, part=0):
        n = RB // parts
        r = rows(jnp.maximum(step, 0) // NG * parts + part, n)
        grp = rows((step + NG) % NG, UNR * DH)
        acc = b_s[r, :] + _dg(
            ot_s[grp, part * n:(part + 1) * n], wo_s[grp, :], TN)
        b_s[r, :] = acc
        o_s[r, :] = acc.astype(bf16)

    def fast_heads(step):
        qb, it = step // NG, step % NG
        n = UNR * NC

        def unit(i):
            dh, c = divmod(i, NC)
            if dh < UNR:
                return qb, it * UNR + dh, c
            return jnp.minimum((step + 1) // NG, NB - 1), (step + 1) % NG * UNR, c

        ss, sv = {}, {}
        zero = pltpu.bitcast(h_s[:8, :128], u32)
        for i in range(n):
            ss[i + SKEW] = scores(*unit(i + SKEW), VK[(i + SKEW) % len(VK)])
            if i == NC - 1:
                project(step - 1)
            _, h, c = unit(i)
            nv = VK[c % len(VK)]
            p = [ss[i] if i >= SKEW else ss_s[i, :KC - nv]]
            if nv:
                p.append(sv[i] if i >= VSKEW else ss_s[i, KC - nv:])
            p = jnp.exp2(jnp.concatenate(p, axis=0))
            j = i + SKEW - n
            if j >= 0:
                ss_s[j, :KC - VK[j % len(VK)]] = ss[i + SKEW]
            deps = []
            for r in range(0, KC, 8):
                l = p[:8] if c == 0 and r == 0 else l + p[r:r + 8]
                if r % (KC // ND) == 8:
                    deps.append(jnp.tile(pltpu.bitcast(l[:, :128], u32) & zero, (VKM // 8, 1)))
            if VK[(i + VSKEW) % len(VK)]:
                sv[i + VSKEW] = vpu_scores(*unit(i + VSKEW), deps)
                j = i + VSKEW - n
                if j >= 0:
                    ss_s[j, KC - VK[j % len(VK)]:] = sv[i + VSKEW]
            ov = _dot(v_chunk(h, c), p.astype(bf16))
            o = ov if c == 0 else o + ov
            if c == NC - 1:
                finish(qb, h, o, l)

    def safe_head(qb, h):
        m = None
        for c in range(NC):
            s = scores(qb, h, c)
            s_s[c] = s
            mc = jnp.max(s.reshape(KC // 8, 8, RB), axis=0)
            m = mc if c == 0 else jnp.maximum(m, mc)
        m = jnp.max(m, axis=0, keepdims=True)
        for c in range(NC):
            p = jnp.exp2(s_s[c] - m)
            ls = jnp.sum(p.reshape(KC // 8, 8, RB), axis=0)
            ov = _dot(v_chunk(h, c), p.astype(bf16))
            l, o = (ls, ov) if c == 0 else (l + ls, o + ov)
        finish(qb, h, o, l)

    def out_cp(i, n=RB, sem=0):
        return pltpu.make_async_copy(o_s.at[rows(i, n)], out_hbm.at[rows(i, n)],
                                     out_sem.at[i + sem])

    def flush(step):
        @pl.when((step > 0) & (step % NG == 0))
        def _():
            out_cp(step // NG - 1).start()

    @pl.when(safe)
    def _():
        @pl.loop(0, NB * NG)
        def _(step):
            fast_heads(step)
            flush(step)

    @pl.when(jnp.logical_not(safe))
    def _():
        @pl.loop(0, NB * NG)
        def _(step):
            project(step - 1)
            flush(step)
            pl.loop(0, UNR)(lambda j: safe_head(step // NG, step % NG * UNR + j))

    last = [out_cp(2 * NB - 2 + j, RB // 2, 1 - NB) for j in range(2)]
    for j in range(2):
        project(NB * NG - 1, 2, j)
        last[j].start()
    for cp in [out_cp(qb) for qb in range(NB - 1)] + last:
        cp.wait()


@jax.jit
def pallas_gated_mix__mha_block__mixer_s_mlp__prompt_kernel(
    A_x: jax.Array,
    A_wqkv: jax.Array,
    A_wo: jax.Array,
    B_x: jax.Array,
    B_w1: jax.Array,
    B_w2: jax.Array,
    B_w3: jax.Array,
    B_w4: jax.Array,
    gate_w: jax.Array,
):
    del B_x
    vm = pltpu.VMEM
    out = pl.pallas_call(
        _kernel,
        out_shape=jax.ShapeDtypeStruct((S, D), bf16),
        in_specs=[pl.BlockSpec(memory_space=pl.ANY)] * 8,
        out_specs=pl.BlockSpec(memory_space=pl.ANY),
        scratch_shapes=[
            vm((S, D), bf16), vm((3, D, D), bf16), vm((D, D), bf16), vm((D, D), bf16),
            vm((D, D), bf16), vm((D, F), bf16), vm((F, D), bf16), vm((1, D), bf16),
            vm((D, D), bf16), vm((D, D), bf16),
            vm((H, S // 2, 128), u32), vm((H, NC * VKM, 128), f32), vm((NB, D, RB), bf16),
            vm((NB, RB // 128, D, 128), f32), vm((NB, D, RB), bf16),
            vm((S + 2 * PAD, D), f32), vm((S, D), f32), vm((NB, 8, RB), f32),
            vm((2, 8, 128), f32), vm((max(SKEW, VSKEW), KC, RB), f32), vm((NC, KC, RB), f32),
            vm((D, RB), bf16), vm((S, D), bf16),
            pltpu.SemaphoreType.DMA((len(XP),)), pltpu.SemaphoreType.DMA((9,)), pltpu.SemaphoreType.DMA((NB + 1,)),
        ],
        compiler_params=pltpu.CompilerParams(vmem_limit_bytes=100 * 2**20),
    )(A_x.reshape(S, D), A_wqkv, A_wo, B_w1, B_w2, B_w3, B_w4, gate_w.reshape(1, D))
    return out.reshape(1, S, D)
```
